```python
import os as _os
_os.environ.setdefault("JAX_PLATFORMS", "cpu")
import jax
import jax.numpy as jnp

def _softmax(x, axis=-1):
    return jax.nn.softmax(x, axis=axis)
def _gelu(x):
    return jax.nn.gelu(x, approximate=True)
def _silu(x):
    return jax.nn.silu(x)
def _sigmoid(x):
    return jax.nn.sigmoid(x)
def _layernorm(x, axis=-1, eps=1e-5):
    m = jnp.mean(x, axis=axis, keepdims=True)
    v = jnp.var(x, axis=axis, keepdims=True)
    return (x - m) / jnp.sqrt(v + eps)
def _scatter_add(tgt, idx, src, axis=0):
    return tgt.at[idx].add(src)
def _segment_sum(src, seg, n):
    return jax.ops.segment_sum(src, seg, n)
class _Rng:
    def __init__(self, key):
        self._k = key
    def _next(self):
        self._k, sub = jax.random.split(self._k)
        return sub
    def normal(self, shape):
        return jax.random.normal(self._next(), shape, dtype=jnp.bfloat16)
    def randint(self, lo, hi, shape):
        return jax.random.randint(self._next(), shape, lo, hi, dtype=jnp.int32)
    def uniform(self, shape, lo=0.0, hi=1.0):
        return jax.random.uniform(self._next(), shape, jnp.bfloat16, lo, hi)
    def permutation(self, n):
        return jax.random.permutation(self._next(), n)


kernel_name = 'parallel_sum__grouped_kv_mqa__dense_activation_silu__prompt'

def setup_inputs():
    _rng = _Rng(jax.random.key(int.from_bytes(__import__("os").urandom(4), "little")))
    _w = (lambda a: (lambda t: t.astype(jnp.bfloat16) if jnp.issubdtype(t.dtype, jnp.floating) else t)(jnp.asarray(a)))
    def _A_setup():
        B, S, D, H = 1, 2048, 512, 32
        Dh = D // H
        return {
            "x": _w((lambda *s: _rng.normal(s) * 0.05)(B, S, D)),
            "wq": _w((lambda *s: _rng.normal(s) * 0.05)(D, H * Dh)),
            "wk": _w((lambda *s: _rng.normal(s) * 0.05)(D, Dh)),
            "wv": _w((lambda *s: _rng.normal(s) * 0.05)(D, Dh)),
            "wo": _w((lambda *s: _rng.normal(s) * 0.05)(H * Dh, D)),
        }
    _A_in = _A_setup()

    def _B_setup():
        B, S, D, F = 1, 2048, 512, 1376
        return {
            "x": _w((lambda *s: _rng.normal(s) * 0.05)(B, S, D)),
            "w1": _w((lambda *s: _rng.normal(s) * 0.05)(D, F) * (D ** -0.5)),
            "w2": _w((lambda *s: _rng.normal(s) * 0.05)(F, D) * (F ** -0.5)),
        }
    _B_in = _B_setup()

    return {
        "A_x": _A_in["x"],
        "A_wq": _A_in["wq"],
        "A_wk": _A_in["wk"],
        "A_wv": _A_in["wv"],
        "A_wo": _A_in["wo"],
        "B_x": _B_in["x"],
        "B_w1": _B_in["w1"],
        "B_w2": _B_in["w2"],
    }

def reference(A_x, A_wq, A_wk, A_wv, A_wo, B_x, B_w1, B_w2):
    def _A_ref(x, wq, wk, wv, wo):
        B, S, D = x.shape
        H = 32
        Dh = D // H
        q = (lambda x, *d: x.transpose(*d))((x @ wq).reshape(B, S, H, Dh), 0, 2, 1, 3)
        k = x @ wk
        v = x @ wv
        scores = jnp.einsum("bhqd,bkd->bhqk", q, k) * (Dh ** -0.5)
        p = _softmax(scores, axis=-1)
        o = jnp.einsum("bhqk,bkd->bhqd", p, v)
        return (lambda x, *d: x.transpose(*d))(o, 0, 2, 1, 3).reshape(B, S, H * Dh) @ wo

    def _B_ref(x, w1, w2):
        h = jnp.einsum("bsd,df->bsf", x, w1)
        h = _silu(h)
        out = jnp.einsum("bsf,fd->bsd", h, w2)
        return out

    x = A_x
    xn = _layernorm(x, axis=-1)
    return x + _A_ref(xn, A_wq, A_wk, A_wv, A_wo) + _B_ref(xn, B_w1, B_w2)
```

```python
import functools
import jax
import jax.numpy as jnp
from jax import lax
import jax.experimental.pallas as pl
import jax.experimental.pallas.tpu as pltpu

BQ = 512
CK = 128
LAG = 2
SKEW = 0
DD = 12
G = 16
U = 5
H = 32
DH = 16
LOG2E = 1.4426950408889634
NT = (((1,), (1,)), ((), ()))


def _ln(x):
    x = x.astype(jnp.float32)
    m = jnp.mean(x, axis=-1, keepdims=True)
    xc = x - m
    v = jnp.mean(xc * xc, axis=-1, keepdims=True)
    return xc * lax.rsqrt(v + 1e-5)


def kernel(x_hbm, wkt_ref, wvt_ref, wq_hbm, wo_hbm, w1t_hbm, w2_hbm, o_ref,
           xn_ref, k_ref, vt_ref, qt_ref, ot_ref, sa_ref, sb_ref,
           wq_ref, wo_ref, w1t_ref, w2_ref, h_ref, x_ref, wk_ref, sems):
    i = pl.program_id(0)
    S, D = x_ref.shape
    F = w2_ref.shape[0]
    NC = S // CK
    cps = [pltpu.make_async_copy(a, b, sems.at[n]) for n, (a, b) in enumerate(
        [(wq_hbm, wq_ref), (w1t_hbm, w1t_ref), (w2_hbm, w2_ref), (wo_hbm, wo_ref)])]

    @pl.when(i == 0)
    def _():
        NX = 4
        XC = S // NX
        xcp = [pltpu.make_async_copy(x_hbm.at[n * XC:(n + 1) * XC], x_ref.at[n * XC:(n + 1) * XC], sems.at[4 + n])
               for n in range(NX)]
        for cp in xcp + cps:
            cp.start()
        wk_ref[...] = jnp.zeros(wk_ref.shape, wk_ref.dtype)
        wk_ref[0:DH, :] = wkt_ref[...]
        for n in range(NX):
            xcp[n].wait()
            rows = slice(n * XC, (n + 1) * XC)
            xn = _ln(x_ref[rows, :]).astype(jnp.bfloat16)
            xn_ref[rows, :] = xn
        xn = xn_ref[...]
        k = lax.dot_general(xn, wk_ref[...], NT, preferred_element_type=jnp.float32)
        k_ref[...] = k.astype(jnp.bfloat16)
        vt = lax.dot_general(wvt_ref[...], xn, NT, preferred_element_type=jnp.float32)
        vt_ref[...] = vt.astype(jnp.bfloat16)
        cps[0].wait()

    r0 = pl.multiple_of(i * BQ, BQ)
    xn = xn_ref[pl.ds(r0, BQ), :]
    q = jnp.dot(xn, wq_ref[...], preferred_element_type=jnp.float32) * (DH ** -0.5 * LOG2E)
    qt_ref[...] = q.T.astype(jnp.bfloat16)

    def qk_chunk(c, qh, s_ref, m, hist=None):
        s = jnp.dot(k_ref[c * CK:(c + 1) * CK, 0:DH], qh, preferred_element_type=jnp.float32)
        s_ref[c * CK:(c + 1) * CK, :] = s
        for j in range(CK // 8):
            sj = s[j * 8:(j + 1) * 8]
            m = sj if m is None else jnp.maximum(m, sj)
            if hist is not None and (j + 1) % (G // 8) == 0:
                hist.append(m)
        return m

    def exp_chunk(c, s_ref, m, l, deps=None):
        if deps is None:
            mm = m[None]
        else:
            ok = m == m
            mm = jnp.stack([m if d is None else jnp.where(ok, m, d) for d in deps for _ in range(G // 8)])
        p = jnp.exp2(s_ref[c * CK:(c + 1) * CK, :].reshape(CK // 8, 8, BQ) - mm)
        lc = p[0] if l is None else l + p[0]
        for j in range(1, CK // 8):
            lc = lc + p[j]
        return lc, p.reshape(CK, BQ).astype(jnp.bfloat16)

    def pv_dot(c, pb, acc):
        a = jnp.dot(vt_ref[:, c * CK:(c + 1) * CK], pb, preferred_element_type=jnp.float32)
        return a if c == 0 else acc + a

    def get_q(h):
        return qt_ref[pl.ds(pl.multiple_of(h * DH, DH), DH), :]

    def fin_max(m):
        return jnp.broadcast_to(jnp.max(m, axis=0, keepdims=True), (8, BQ))

    def finish(h, la):
        ot_ref[pl.ds(pl.multiple_of(h * DH, DH), DH), :] = la[1] / jnp.sum(la[0], axis=0, keepdims=True)

    def stage(h, prev, m_cur, s_cur, s_nxt, do_qk=True, extra=None):
        m_n = None
        l = acc = None
        pend = None
        if prev is not None:
            m_p, l_p, acc_p = prev
        if do_qk:
            qh = get_q(h + 1)
        pend = {}
        hist = []
        R = CK // G
        for c in range(NC + SKEW):
            if do_qk and c < NC:
                m_n = qk_chunk(c, qh, s_nxt, m_n, hist)
            if extra is not None:
                extra(c)
            t = c - LAG
            if c < NC:
                deps = [hist[c * R + j - DD] if c * R + j >= DD else None for j in range(R)] if do_qk else None
                if t < 0:
                    if prev is not None:
                        l_p, pend[t] = exp_chunk(NC + t, s_nxt, m_p, l_p, deps)
                else:
                    l, pend[t] = exp_chunk(t, s_cur, m_cur, l, deps)
            t = t - SKEW
            if t in pend:
                pb = pend.pop(t)
                if t < 0:
                    acc_p = pv_dot(NC + t, pb, acc_p)
                    if t == -1:
                        finish(h - 1, (l_p, acc_p))
                else:
                    acc = pv_dot(t, pb, acc)
        return (m_cur, l, acc), (fin_max(m_n) if do_qk else None)

    m0 = None
    q0 = get_q(0)
    for c in range(NC):
        m0 = qk_chunk(c, q0, sa_ref, m0)
    m0 = fin_max(m0)
    carry = stage(0, None, m0, sa_ref, sb_ref)

    def body(j, carry):
        for u in range(U):
            carry = stage(2 * (j * U + u) + 1, carry[0], carry[1], sb_ref, sa_ref)
            carry = stage(2 * (j * U + u) + 2, carry[0], carry[1], sa_ref, sb_ref)
        return carry

    carry = lax.fori_loop(0, (H // 2 - 1) // U, body, carry)

    @pl.when(i == 0)
    def _():
        for cp in cps[1:]:
            cp.wait()

    xn = xn_ref[pl.ds(r0, BQ), :]
    FC = 256
    nf = pl.cdiv(F, FC)

    def ffn1(c):
        if c % 2 == 0 and c // 2 < nf:
            f0 = (c // 2) * FC
            f1 = min(F, f0 + FC)
            h1 = lax.dot_general(xn, w1t_ref[f0:f1, :], NT, preferred_element_type=jnp.float32)
            hh = 0.5 * h1
            h_ref[:, f0:f1] = (hh * jnp.tanh(hh) + hh).astype(jnp.bfloat16)

    prev, _ = stage(H - 1, carry[0], carry[1], sb_ref, sa_ref, do_qk=False, extra=ffn1)
    for t in range(-LAG, 0):
        l, pb = exp_chunk(NC + t, sb_ref, prev[0], prev[1])
        prev = (prev[0], l, pv_dot(NC + t, pb, prev[2]))
    finish(H - 1, prev[1:])

    b = jnp.dot(h_ref[...], w2_ref[...], preferred_element_type=jnp.float32)
    o = ot_ref[...].T.astype(jnp.bfloat16)
    a = jnp.dot(o, wo_ref[...], preferred_element_type=jnp.float32)
    o_ref[...] = (x_ref[pl.ds(r0, BQ), :].astype(jnp.float32) + a + b).astype(o_ref.dtype)


@jax.jit
def pallas_parallel_sum__grouped_kv_mqa__dense_activation_silu__prompt_kernel(
        A_x, A_wq, A_wk, A_wv, A_wo, B_x, B_w1, B_w2):
    B, S, D = A_x.shape
    F = B_w1.shape[1]
    x = A_x.reshape(S, D)
    full = lambda shape: pl.BlockSpec(shape, lambda i: (0,) * len(shape))
    hbm = pl.BlockSpec(memory_space=pl.ANY)
    out = pl.pallas_call(
        kernel,
        grid=(S // BQ,),
        in_specs=[hbm, full((DH, D)), full((DH, D)), hbm, hbm, hbm, hbm],
        out_specs=pl.BlockSpec((BQ, D), lambda i: (i, 0)),
        out_shape=jax.ShapeDtypeStruct((S, D), A_x.dtype),
        scratch_shapes=[
            pltpu.VMEM((S, D), jnp.bfloat16),
            pltpu.VMEM((S, 128), jnp.bfloat16),
            pltpu.VMEM((DH, S), jnp.bfloat16),
            pltpu.VMEM((D, BQ), jnp.bfloat16),
            pltpu.VMEM((D, BQ), jnp.float32),
            pltpu.VMEM((S, BQ), jnp.float32),
            pltpu.VMEM((S, BQ), jnp.float32),
            pltpu.VMEM((D, D), jnp.bfloat16),
            pltpu.VMEM((D, D), jnp.bfloat16),
            pltpu.VMEM((F, D), jnp.bfloat16),
            pltpu.VMEM((F, D), jnp.bfloat16),
            pltpu.VMEM((BQ, F), jnp.bfloat16),
            pltpu.VMEM((S, D), jnp.bfloat16),
            pltpu.VMEM((128, D), jnp.bfloat16),
            pltpu.SemaphoreType.DMA((12,)),
        ],
        compiler_params=pltpu.CompilerParams(
            dimension_semantics=("arbitrary",), vmem_limit_bytes=100 * 1024 * 1024),
    )(x, A_wk.T, A_wv.T, A_wq, A_wo, B_w1.T, B_w2)
    return out.reshape(B, S, D)
```
